```python
import jax
import jax.numpy as jnp

def _softmax(x, axis=-1):
    return jax.nn.softmax(x, axis=axis)

def _gelu(x):
    return jax.nn.gelu(x, approximate=True)

def _silu(x):
    return jax.nn.silu(x)

def _sigmoid(x):
    return jax.nn.sigmoid(x)

def _layernorm(x, axis=-1, eps=1e-05):
    m = jnp.mean(x, axis=axis, keepdims=True)
    v = jnp.var(x, axis=axis, keepdims=True)
    return (x - m) / jnp.sqrt(v + eps)

def _scatter_add(tgt, idx, src, axis=0):
    return tgt.at[idx].add(src)

def _segment_sum(src, seg, n):
    return jax.ops.segment_sum(src, seg, n)

class _Rng:

    def __init__(self, key):
        self._k = key

    def _next(self):
        self._k, sub = jax.random.split(self._k)
        return sub

    def normal(self, shape):
        return jax.random.normal(self._next(), shape, dtype=jnp.bfloat16)

    def randint(self, lo, hi, shape):
        return jax.random.randint(self._next(), shape, lo, hi, dtype=jnp.int32)

    def uniform(self, shape, lo=0.0, hi=1.0):
        return jax.random.uniform(self._next(), shape, jnp.bfloat16, lo, hi)

    def permutation(self, n):
        return jax.random.permutation(self._next(), n)
kernel_name = 'adaLN_cond__sliding_block_cached__geglu_ffn__decode'

def setup_inputs():
    _rng = _Rng(jax.random.key(int.from_bytes(__import__("os").urandom(4), "little")))
    _w = lambda a: (lambda t: t.astype(jnp.bfloat16) if jnp.issubdtype(t.dtype, jnp.floating) else t)(jnp.asarray(a))

    def _A_setup():
        B, Sq, D = (1, 1, 640)
        Hq, Hkv, Sk, Dh = (32, 32, 32768, 192)
        assert Hq % Hkv == 0, (Hq, Hkv)
        return {'x': _w((lambda *s: _rng.normal(s) * 0.05)(B, Sq, D)), 'k_cache': _w((lambda *s: _rng.normal(s) * 0.05)(B, Hkv, Sk, Dh)), 'v_cache': _w((lambda *s: _rng.normal(s) * 0.05)(B, Hkv, Sk, Dh)), 'wq': _w((lambda *s: _rng.normal(s) * 0.05)(D, Hq * Dh) * D ** (-0.5)), 'wo': _w((lambda *s: _rng.normal(s) * 0.05)(Hq * Dh, D) * (Hq * Dh) ** (-0.5))}
    _A_in = _A_setup()

    def _B_setup():
        B, S, D, F = (1, 1, 640, 1536)
        return {'x': _w((lambda *s: _rng.normal(s) * 0.05)(B, S, D)), 'w_gate': _w((lambda *s: _rng.normal(s) * 0.05)(D, F)), 'w_up': _w((lambda *s: _rng.normal(s) * 0.05)(D, F)), 'w_down': _w((lambda *s: _rng.normal(s) * 0.05)(F, D))}
    _B_in = _B_setup()
    return {'A_x': _A_in['x'], 'A_k_cache': _A_in['k_cache'], 'A_v_cache': _A_in['v_cache'], 'A_wq': _A_in['wq'], 'A_wo': _A_in['wo'], 'B_x': _B_in['x'], 'B_w_gate': _B_in['w_gate'], 'B_w_up': _B_in['w_up'], 'B_w_down': _B_in['w_down'], 'c': _w((lambda *s: _rng.normal(s) * 0.05)(1, 640)), 'w_mod': _w((lambda *s: _rng.normal(s) * 0.05)(640, 6 * 640) * 640 ** (-0.5))}

def reference(A_x, A_k_cache, A_v_cache, A_wq, A_wo, B_x, B_w_gate, B_w_up, B_w_down, c, w_mod):

    def _A_ref(x, k_cache, v_cache, wq, wo):
        B, Sq, D = x.shape
        Hq, Dh = (32, 192)
        Hkv, Sk = (k_cache.shape[1], k_cache.shape[2])
        W = min(4096, max(256, Sk // 4))
        rep = Hq // Hkv
        q = (lambda x, *d: x.transpose(*d))((x @ wq).reshape(B, Sq, Hq, Dh), 0, 2, 1, 3)
        k = jnp.repeat(k_cache[:, :, Sk - W:, :], rep, axis=1)
        v = jnp.repeat(v_cache[:, :, Sk - W:, :], rep, axis=1)
        scores = jnp.einsum('bhqd,bhkd->bhqk', q, k) * Dh ** (-0.5)
        p = _softmax(scores, axis=-1)
        o = jnp.einsum('bhqk,bhkd->bhqd', p, v)
        return (lambda x, *d: x.transpose(*d))(o, 0, 2, 1, 3).reshape(B, Sq, Hq * Dh) @ wo

    def _B_ref(x, w_gate, w_up, w_down):
        return _gelu(x @ w_gate) * (x @ w_up) @ w_down
    x = A_x
    mod = (_silu(c) @ w_mod).reshape(c.shape[0], 6, 1, -1)
    sa, ca, ga, sb, cb, gb = (mod[:, 0].copy(), mod[:, 1].copy(), mod[:, 2].copy(), mod[:, 3].copy(), mod[:, 4].copy(), mod[:, 5].copy())
    h = _layernorm(x, axis=-1) * (1 + ca) + sa
    x = x + ga * _A_ref(h, A_k_cache, A_v_cache, A_wq, A_wo)
    h = _layernorm(x, axis=-1) * (1 + cb) + sb
    x = x + gb * _B_ref(h, B_w_gate, B_w_up, B_w_down)
    return x
```

```python
import functools

import jax
import jax.numpy as jnp
import numpy as np
from jax import lax
from jax.experimental import pallas as pl
from jax.experimental.pallas import tpu as pltpu


def _ln(x, eps=1e-5):
    m = jnp.mean(x, axis=-1, keepdims=True)
    d = x - m
    v = jnp.mean(d * d, axis=-1, keepdims=True)
    return d / jnp.sqrt(v + eps)


def _gelu(x):
    c = float(np.sqrt(2.0 / np.pi))
    return 0.5 * x * (1.0 + jnp.tanh(c * (x + 0.044715 * (x * x * x))))


def _dot(a, b):
    return jnp.dot(a, b, preferred_element_type=jnp.float32)


def _dot_nt(a, b):
    return lax.dot_general(a, b, (((1,), (1,)), ((), ())), preferred_element_type=jnp.float32)


def make_kernel(D, H, Dh, Sk, W, F, HP, R, FC):
    NP = H // HP
    G = HP * Dh
    S0 = Sk - W
    NF = F // FC
    scale = float(Dh) ** -0.5
    bf16 = jnp.bfloat16

    def kernel(x_hbm, c_hbm, kT_hbm, vT_hbm, wq_hbm, wo_hbm, wg_hbm, wu_hbm, wd_hbm, wmod_hbm,
               o_ref,
               x_v, c_v, wmod_v, wq_v, k_v, v_v, wo_v, wg_v, wu_v, wd_v,
               sem_s, sem_q, sem_k, sem_v, sem_o, sem_f):

        def cp_q(p, slot):
            off = pl.multiple_of(p * G, 128)
            return pltpu.make_async_copy(wq_hbm.at[:, pl.ds(off, G)], wq_v.at[slot], sem_q.at[slot])

        def cp_k(p, slot):
            off = pl.multiple_of(p * G, 128)
            return pltpu.make_async_copy(kT_hbm.at[pl.ds(off, G), pl.ds(S0, W)], k_v.at[slot], sem_k.at[slot])

        def cp_v(p, slot):
            off = pl.multiple_of(p * G, 128)
            return pltpu.make_async_copy(vT_hbm.at[pl.ds(off, G), pl.ds(S0, W)], v_v.at[slot], sem_v.at[slot])

        def cp_o(p, slot):
            off = pl.multiple_of(p * G, 128)
            return pltpu.make_async_copy(wo_hbm.at[pl.ds(off, G), :], wo_v.at[slot], sem_o.at[slot])

        def cp_g(j):
            return pltpu.make_async_copy(wg_hbm.at[:, pl.ds(j * FC, FC)], wg_v.at[j], sem_f.at[0, j])

        def cp_u(j):
            return pltpu.make_async_copy(wu_hbm.at[:, pl.ds(j * FC, FC)], wu_v.at[j], sem_f.at[1, j])

        def cp_d(j):
            return pltpu.make_async_copy(wd_hbm.at[pl.ds(j * FC, FC), :], wd_v.at[j], sem_f.at[2, j])

        cp_c = pltpu.make_async_copy(c_hbm, c_v, sem_s.at[0])
        cp_x = pltpu.make_async_copy(x_hbm, x_v, sem_s.at[1])
        cp_m = pltpu.make_async_copy(wmod_hbm, wmod_v, sem_s.at[2])

        cp_c.start()
        cp_x.start()
        cp_m.start()
        for r in range(R):
            cp_q(r, r).start()
            cp_k(r, r).start()
            cp_v(r, r).start()
            cp_o(r, r).start()

        cp_c.wait()
        cf = c_v[...].astype(jnp.float32)
        sc = (cf * jax.nn.sigmoid(cf)).astype(bf16)
        cp_x.wait()
        xf = x_v[...].astype(jnp.float32)
        lnx = _ln(xf)
        cp_m.wait()
        mod = _dot(sc, wmod_v[...])
        sa = mod[:, 0 * D:1 * D]
        ca = mod[:, 1 * D:2 * D]
        ga = mod[:, 2 * D:3 * D]
        sb = mod[:, 3 * D:4 * D]
        cb = mod[:, 4 * D:5 * D]
        gb = mod[:, 5 * D:6 * D]
        h = (lnx * (1.0 + ca) + sa).astype(bf16)

        rows = lax.broadcasted_iota(jnp.int32, (8, G), 0)
        cols = lax.broadcasted_iota(jnp.int32, (8, G), 1)
        mask = (cols >= rows * Dh) & (cols < (rows + 1) * Dh)

        def body(p, acc):
            slot = lax.rem(p, R)
            nxt = jnp.minimum(p + R, NP - 1)
            has_next = p + R < NP

            cp_q(p, slot).wait()
            q = _dot(h, wq_v[slot])

            @pl.when(has_next)
            def _():
                cp_q(nxt, slot).start()

            qb = jnp.where(mask, jnp.broadcast_to(q.astype(bf16).astype(jnp.float32), (8, G)), 0.0).astype(bf16)
            cp_k(p, slot).wait()
            s = _dot(qb, k_v[slot]) * scale

            @pl.when(has_next)
            def _():
                cp_k(nxt, slot).start()

            m = jnp.max(s, axis=-1, keepdims=True)
            e = jnp.exp(s - m)
            l = jnp.sum(e, axis=-1, keepdims=True)
            cp_v(p, slot).wait()
            o = _dot_nt(e.astype(bf16), v_v[slot])

            @pl.when(has_next)
            def _():
                cp_v(nxt, slot).start()

            o = jnp.where(mask, o / l, 0.0).astype(bf16)
            cp_o(p, slot).wait()
            acc = acc + _dot(o, wo_v[slot])

            @pl.when(has_next)
            def _():
                cp_o(nxt, slot).start()

            @pl.when(p == NP - R)
            def _():
                for j in range(NF):
                    cp_g(j).start()
                    cp_u(j).start()
                    cp_d(j).start()

            return acc

        acc = lax.fori_loop(0, NP, body, jnp.zeros((8, D), jnp.float32))
        attn = jnp.sum(acc, axis=0, keepdims=True)
        x1 = xf + ga * attn
        h2 = (_ln(x1) * (1.0 + cb) + sb).astype(bf16)
        y = jnp.zeros((1, D), jnp.float32)
        for j in range(NF):
            cp_g(j).wait()
            g = _dot(h2, wg_v[j])
            cp_u(j).wait()
            u = _dot(h2, wu_v[j])
            a = (_gelu(g) * u).astype(bf16)
            cp_d(j).wait()
            y = y + _dot(a, wd_v[j])
        o_ref[...] = (x1 + gb * y).astype(o_ref.dtype)

    return kernel


HP = 2
R = 2
FC = 512


def _build(HP, R, FC):
    def fn(A_x, A_k_cache, A_v_cache, A_wq, A_wo, B_x, B_w_gate, B_w_up, B_w_down, c, w_mod):
        B, Sq, D = A_x.shape
        _, H, Sk, Dh = A_k_cache.shape
        W = min(4096, max(256, Sk // 4))
        F = B_w_gate.shape[1]
        G = HP * Dh
        NF = F // FC
        bf16 = jnp.bfloat16
        kT = jnp.swapaxes(A_k_cache, 2, 3).reshape(H * Dh, Sk)
        vT = jnp.swapaxes(A_v_cache, 2, 3).reshape(H * Dh, Sk)
        x2 = A_x.reshape(1, D)
        kern = make_kernel(D, H, Dh, Sk, W, F, HP, R, FC)
        any_spec = pl.BlockSpec(memory_space=pl.ANY)
        out = pl.pallas_call(
            kern,
            out_shape=jax.ShapeDtypeStruct((1, D), A_x.dtype),
            in_specs=[any_spec] * 10,
            out_specs=pl.BlockSpec(memory_space=pltpu.VMEM),
            scratch_shapes=[
                pltpu.VMEM((1, D), bf16),
                pltpu.VMEM((1, D), bf16),
                pltpu.VMEM((D, 6 * D), bf16),
                pltpu.VMEM((R, D, G), bf16),
                pltpu.VMEM((R, G, W), bf16),
                pltpu.VMEM((R, G, W), bf16),
                pltpu.VMEM((R, G, D), bf16),
                pltpu.VMEM((NF, D, FC), bf16),
                pltpu.VMEM((NF, D, FC), bf16),
                pltpu.VMEM((NF, FC, D), bf16),
                pltpu.SemaphoreType.DMA((3,)),
                pltpu.SemaphoreType.DMA((R,)),
                pltpu.SemaphoreType.DMA((R,)),
                pltpu.SemaphoreType.DMA((R,)),
                pltpu.SemaphoreType.DMA((R,)),
                pltpu.SemaphoreType.DMA((3, NF)),
            ],
            compiler_params=pltpu.CompilerParams(vmem_limit_bytes=100 * 1024 * 1024),
        )(x2, c, kT, vT, A_wq, A_wo, B_w_gate, B_w_up, B_w_down, w_mod)
        return out.reshape(B, Sq, D)

    return fn


@jax.jit
def pallas_adaLN_cond__sliding_block_cached__geglu_ffn__decode_kernel(
    A_x: jax.Array,
    A_k_cache: jax.Array,
    A_v_cache: jax.Array,
    A_wq: jax.Array,
    A_wo: jax.Array,
    B_x: jax.Array,
    B_w_gate: jax.Array,
    B_w_up: jax.Array,
    B_w_down: jax.Array,
    c: jax.Array,
    w_mod: jax.Array,
):
    return _build(HP, R, FC)(A_x, A_k_cache, A_v_cache, A_wq, A_wo, B_x, B_w_gate, B_w_up, B_w_down, c, w_mod)
```

```python
import functools

import jax
import jax.numpy as jnp
import numpy as np
from jax import lax
from jax.experimental import pallas as pl
from jax.experimental.pallas import tpu as pltpu


def _ln(x, eps=1e-5):
    m = jnp.mean(x, axis=-1, keepdims=True)
    d = x - m
    v = jnp.mean(d * d, axis=-1, keepdims=True)
    return d / jnp.sqrt(v + eps)


def _gelu(x):
    c = float(np.sqrt(2.0 / np.pi))
    return 0.5 * x * (1.0 + jnp.tanh(c * (x + 0.044715 * (x * x * x))))


def _dot(a, b):
    return jnp.dot(a, b, preferred_element_type=jnp.float32)


def _dot_nt(a, b):
    return lax.dot_general(a, b, (((1,), (1,)), ((), ())), preferred_element_type=jnp.float32)


def _loop(lo, hi, fn):
    if hi > lo:
        lax.fori_loop(lo, hi, lambda i, c: (fn(i), c)[1], 0)


def make_kernel(D, H, Dh, Sk, W, F, cfg):
    HP, R = 2, 2
    NP = H // HP
    G = HP * Dh
    S0 = Sk - W
    scale = float(Dh) ** -0.5
    bf16 = jnp.bfloat16
    ksr, ksc = cfg["kv"]
    NC = W // ksc
    NB = G // ksr
    cA, cB, cC = cfg["split"]
    qsr = cfg["q"]
    osr = cfg["o"]
    msr, msc = cfg["m"]
    gsr, gsc = cfg["g"]
    dsr = cfg["d"]
    FCs = cfg["fchunks"]
    foffs = np.cumsum([0] + list(FCs))[:-1].tolist()
    NF = len(FCs)
    nocompute = cfg.get("nocompute", False)
    qt0 = cfg.get("qt0", 0)

    ffn = []
    for j in range(NF):
        for nm in "gu":
            for r0 in range(0, D, gsr):
                for c0 in range(0, FCs[j], gsc):
                    ffn.append((nm, j, r0, min(gsr, D - r0), c0, min(gsc, FCs[j] - c0)))
        for r0 in range(0, FCs[j], dsr):
            ffn.append(("d", j, r0, min(dsr, FCs[j] - r0), 0, D))
    fA, fB, fC = cfg["fsplit"]

    def kernel(x_hbm, c_hbm, kT_hbm, vT_hbm, wq_hbm, wo_hbm, wg_hbm, wu_hbm, wd_hbm, wmod_hbm,
               o_ref,
               x_v, c_v, wmod_v, wq_v, k_v, v_v, wo_v, *rest):
        wg_v = rest[0:NF]
        wu_v = rest[NF:2 * NF]
        wd_v = rest[2 * NF:3 * NF]
        sem_s, sem_p, sem_f = rest[3 * NF:]

        def wait_buf(buf, sem):
            pltpu.make_async_copy(buf, buf, sem).wait()

        def issue_q(p, slot):
            off = pl.multiple_of(p * G, 128)
            for i, r0 in enumerate(range(0, D, qsr)):
                pltpu.make_async_copy(wq_hbm.at[pl.ds(r0, qsr), pl.ds(off, G)], wq_v.at[slot, pl.ds(r0, qsr), :],
                                      sem_p.at[0, slot]).start(priority=(i + qt0) % 2)

        def issue_o(p, slot):
            off = pl.multiple_of(p * G, 128)
            for i, r0 in enumerate(range(0, G, osr)):
                pltpu.make_async_copy(wo_hbm.at[pl.ds(off + r0, osr), :], wo_v.at[slot, pl.ds(r0, osr), :],
                                      sem_p.at[3, slot]).start(priority=i % 2)

        def issue_kv(p, slot, lo, hi):
            off = pl.multiple_of(p * G, 128)

            def one(cb):
                c0 = pl.multiple_of(cb * ksc, 128)
                for b in range(NB):
                    r0 = b * ksr
                    for t, (src, dst, sem) in enumerate(((kT_hbm, k_v, sem_p.at[1, slot]), (vT_hbm, v_v, sem_p.at[2, slot]))):
                        pltpu.make_async_copy(src.at[pl.ds(off + r0, ksr), pl.ds(S0 + c0, ksc)],
                                              dst.at[slot, pl.ds(r0, ksr), pl.ds(c0, ksc)], sem).start(priority=t)
            _loop(lo, hi, one)

        def issue_m():
            ncol = (6 * D) // msc
            grp = 2 * msr

            def one(i):
                k = 0
                for rr in range(2):
                    r0 = pl.multiple_of(i * grp + rr * msr, msr)
                    for cc in range(ncol):
                        pltpu.make_async_copy(wmod_hbm.at[pl.ds(r0, msr), pl.ds(cc * msc, msc)],
                                              wmod_v.at[pl.ds(r0, msr), pl.ds(cc * msc, msc)],
                                              sem_s.at[2]).start(priority=k % 2)
                        k += 1
            _loop(0, D // grp, one)

        def issue_ffn(lo, hi):
            for k in range(lo, min(hi, len(ffn))):
                nm, j, r0, nr, c0, nc = ffn[k]
                if nm == "g":
                    src = wg_hbm.at[pl.ds(r0, nr), pl.ds(foffs[j] + c0, nc)]
                    dst = wg_v[j].at[pl.ds(r0, nr), pl.ds(c0, nc)]
                    sem = sem_f.at[0, j]
                elif nm == "u":
                    src = wu_hbm.at[pl.ds(r0, nr), pl.ds(foffs[j] + c0, nc)]
                    dst = wu_v[j].at[pl.ds(r0, nr), pl.ds(c0, nc)]
                    sem = sem_f.at[1, j]
                else:
                    src = wd_hbm.at[pl.ds(foffs[j] + r0, nr), :]
                    dst = wd_v[j].at[pl.ds(r0, nr), :]
                    sem = sem_f.at[2, j]
                pltpu.make_async_copy(src, dst, sem).start(priority=k % 2)

        def part_a(p, slot):
            issue_q(p, slot)
            issue_kv(p, slot, 0, cA)

        def part_b(p, slot):
            issue_kv(p, slot, cA, cB)

        def part_c(p, slot):
            issue_kv(p, slot, cB, cC)

        def part_d(p, slot):
            issue_kv(p, slot, cC, NC)
            issue_o(p, slot)

        cp_c = pltpu.make_async_copy(c_hbm, c_v, sem_s.at[0])
        cp_x = pltpu.make_async_copy(x_hbm, x_v, sem_s.at[1])
        cp_c.start()
        cp_x.start()
        issue_m()
        part_a(0, 0)

        def run_once(fn):
            _loop(0, 1, lambda i: fn())

        cp_c.wait()
        cf = c_v[...].astype(jnp.float32)
        sc = (cf * jax.nn.sigmoid(cf)).astype(bf16)
        cp_x.wait()
        xf = x_v[...].astype(jnp.float32)
        lnx = _ln(xf)
        wait_buf(wmod_v, sem_s.at[2])
        mod = _dot(sc, wmod_v[...])
        sa = mod[:, 0 * D:1 * D]
        ca = mod[:, 1 * D:2 * D]
        ga = mod[:, 2 * D:3 * D]
        sb = mod[:, 3 * D:4 * D]
        cb = mod[:, 4 * D:5 * D]
        gb = mod[:, 5 * D:6 * D]
        h = (lnx * (1.0 + ca) + sa).astype(bf16)

        part_b(0, 0)
        part_c(0, 0)
        part_d(0, 0)
        part_a(1, 1)

        rows = lax.broadcasted_iota(jnp.int32, (8, G), 0)
        cols = lax.broadcasted_iota(jnp.int32, (8, G), 1)
        mask = (cols >= rows * Dh) & (cols < (rows + 1) * Dh)

        def body(p, acc):
            slot = lax.rem(p, R)
            nslot = 1 - slot
            p1 = jnp.minimum(p + 1, NP - 1)
            p2 = jnp.minimum(p + 2, NP - 1)

            def hook(pair_fn, flo, fhi):
                @pl.when(p + 1 < NP)
                def _():
                    pair_fn(p1, nslot)

                @pl.when(p + 1 == NP)
                def _():
                    issue_ffn(flo, fhi)

            wait_buf(wq_v.at[slot], sem_p.at[0, slot])
            if nocompute:
                wait_buf(k_v.at[slot], sem_p.at[1, slot])
                hook(part_b, fA, fB)
                wait_buf(v_v.at[slot], sem_p.at[2, slot])
                hook(part_c, fB, fC)
                wait_buf(wo_v.at[slot], sem_p.at[3, slot])
                acc = acc + k_v[slot, 0:16, 0:D].astype(jnp.float32)[0:8]
            else:
                q = _dot(h, wq_v[slot])
                qb = jnp.where(mask, jnp.broadcast_to(q, (8, G)), 0.0).astype(bf16)
                wait_buf(k_v.at[slot], sem_p.at[1, slot])
                s = _dot(qb, k_v[slot]) * scale
                m = jnp.max(s, axis=-1, keepdims=True)
                e = jnp.exp(s - m)
                l = jnp.sum(e, axis=-1, keepdims=True)
                hook(part_b, fA, fB)
                wait_buf(v_v.at[slot], sem_p.at[2, slot])
                o = _dot_nt(e.astype(bf16), v_v[slot])
                o = jnp.where(mask, o / l, 0.0).astype(bf16)
                hook(part_c, fB, fC)
                wait_buf(wo_v.at[slot], sem_p.at[3, slot])
                acc = acc + _dot(o, wo_v[slot])
            hook(part_d, fC, len(ffn))

            @pl.when(p + 2 < NP)
            def _():
                part_a(p2, slot)

            @pl.when(p + 2 == NP)
            def _():
                issue_ffn(0, fA)

            return acc

        acc = lax.fori_loop(0, NP, body, jnp.zeros((8, D), jnp.float32))
        attn = jnp.sum(acc, axis=0, keepdims=True)
        x1 = xf + ga * attn
        h2 = (_ln(x1) * (1.0 + cb) + sb).astype(bf16)
        y = jnp.zeros((1, D), jnp.float32)
        for j in range(NF):
            wait_buf(wg_v[j], sem_f.at[0, j])
            wait = wait_buf
            if nocompute:
                wait(wu_v[j], sem_f.at[1, j])
                wait(wd_v[j], sem_f.at[2, j])
                continue
            g = _dot(h2, wg_v[j][...])
            wait(wu_v[j], sem_f.at[1, j])
            u = _dot(h2, wu_v[j][...])
            a = (_gelu(g) * u).astype(bf16)
            wait(wd_v[j], sem_f.at[2, j])
            y = y + _dot(a, wd_v[j][...])
        o_ref[...] = (x1 + gb * y).astype(o_ref.dtype)

    return kernel, FCs


DEFAULT = dict(kv=(64, 256), split=(5, 8, 11), q=64, o=32, m=(8, 1280), g=(64, 256), d=32,
               fchunks=(512, 512, 512), fsplit=(70, 106, 142))


def _build(**over):
    cfg = dict(DEFAULT)
    cfg.update(over)

    def fn(A_x, A_k_cache, A_v_cache, A_wq, A_wo, B_x, B_w_gate, B_w_up, B_w_down, c, w_mod):
        B, Sq, D = A_x.shape
        _, H, Sk, Dh = A_k_cache.shape
        W = min(4096, max(256, Sk // 4))
        F = B_w_gate.shape[1]
        G = 2 * Dh
        R = 2
        bf16 = jnp.bfloat16
        kT = jnp.swapaxes(A_k_cache, 2, 3).reshape(H * Dh, Sk)
        vT = jnp.swapaxes(A_v_cache, 2, 3).reshape(H * Dh, Sk)
        x2 = A_x.reshape(1, D)
        kern, FCs = make_kernel(D, H, Dh, Sk, W, F, cfg)
        NF = len(FCs)
        any_spec = pl.BlockSpec(memory_space=pl.ANY)
        out = pl.pallas_call(
            kern,
            out_shape=jax.ShapeDtypeStruct((1, D), A_x.dtype),
            in_specs=[any_spec] * 10,
            out_specs=pl.BlockSpec(memory_space=pltpu.VMEM),
            scratch_shapes=[
                pltpu.VMEM((1, D), bf16),
                pltpu.VMEM((1, D), bf16),
                pltpu.VMEM((D, 6 * D), bf16),
                pltpu.VMEM((R, D, G), bf16),
                pltpu.VMEM((R, G, W), bf16),
                pltpu.VMEM((R, G, W), bf16),
                pltpu.VMEM((R, G, D), bf16),
            ] + [pltpu.VMEM((D, fc), bf16) for fc in FCs]
              + [pltpu.VMEM((D, fc), bf16) for fc in FCs]
              + [pltpu.VMEM((fc, D), bf16) for fc in FCs]
              + [
                pltpu.SemaphoreType.DMA((3,)),
                pltpu.SemaphoreType.DMA((4, R)),
                pltpu.SemaphoreType.DMA((3, NF)),
            ],
            compiler_params=pltpu.CompilerParams(vmem_limit_bytes=100 * 1024 * 1024,
                                                 disable_bounds_checks=True,
                                                 disable_semaphore_checks=True),
        )(x2, c, kT, vT, A_wq, A_wo, B_w_gate, B_w_up, B_w_down, w_mod)
        return out.reshape(B, Sq, D)

    return fn


@jax.jit
def pallas_adaLN_cond__sliding_block_cached__geglu_ffn__decode_kernel(
    A_x: jax.Array,
    A_k_cache: jax.Array,
    A_v_cache: jax.Array,
    A_wq: jax.Array,
    A_wo: jax.Array,
    B_x: jax.Array,
    B_w_gate: jax.Array,
    B_w_up: jax.Array,
    B_w_down: jax.Array,
    c: jax.Array,
    w_mod: jax.Array,
):
    del B_x
    return _build(kv=(32, 512), split=(2, 4, 5))(A_x, A_k_cache, A_v_cache, A_wq, A_wo, None, B_w_gate, B_w_up, B_w_down, c, w_mod)
```

```python
import contextlib

import jax
import jax.numpy as jnp
import numpy as np
from jax import lax
from jax.experimental import pallas as pl
from jax.experimental.pallas import tpu as pltpu


def _ln(x, eps=1e-5):
    m = jnp.mean(x, axis=-1, keepdims=True)
    d = x - m
    v = jnp.mean(d * d, axis=-1, keepdims=True)
    return d / jnp.sqrt(v + eps)


def _gelu(x):
    c = float(np.sqrt(2.0 / np.pi))
    return 0.5 * x * (1.0 + jnp.tanh(c * (x + 0.044715 * (x * x * x))))


def _dot(a, b):
    return jnp.dot(a, b, preferred_element_type=jnp.float32)


def _dot_nt(a, b):
    return lax.dot_general(a, b, (((1,), (1,)), ((), ())), preferred_element_type=jnp.float32)


def _loop(lo, hi, fn):
    if hi > lo:
        lax.fori_loop(lo, hi, lambda i, c: (fn(i), c)[1], 0)


def make_kernel(D, H, Dh, Sk, W, F, cfg):
    HP, R = 2, 3
    NP = H // HP
    G = HP * Dh
    HD = H * Dh
    S0 = Sk - W
    scale = float(Dh) ** -0.5
    bf16 = jnp.bfloat16
    ksr, ksc = cfg["kv"]
    NC = W // ksc
    NB = G // ksr
    NS = 2 * NC
    assert NB % 2 == 0
    HB = NB // 2
    nocompute = cfg.get("nocompute", False)
    ND = cfg["nd"]
    DR = F // ND
    NO = cfg["no"]
    scope = (lambda n: jax.named_scope(n)) if cfg.get("scopes") else (lambda n: contextlib.nullcontext())

    def kernel(x_hbm, c_hbm, kT_hbm, vT_hbm, wq_hbm, wo_hbm, wg_hbm, wu_hbm, wd_hbm, wmod_hbm,
               o_ref,
               x_v, c_v, wmod_v, wq_v, k_v, v_v, wo_v, wgu_v, wd_v, q_v, s_v, gu_v, a_v,
               sem_s, sem_p, sem_gu, sem_d):

        def wait_buf(buf, sem):
            pltpu.make_async_copy(buf, buf, sem).wait()

        def copy(src, dst, sem, t):
            pltpu.make_async_copy(src, dst, sem).start(priority=t)

        def stream_step(arrs, row0, rows, cols, sr, sc, S, j, drow0=None):
            reg = rows // S
            assert reg * S == rows and reg % sr == 0 and cols % sc == 0
            k = 0
            for cc in range(cols // sc):
                for s in range(S):
                    r = s * reg + j * sr
                    r0 = row0 + r
                    d0 = r0 if drow0 is None else drow0 + r
                    if not isinstance(r0, int):
                        r0 = pl.multiple_of(r0, 8)
                    if not isinstance(d0, int):
                        d0 = pl.multiple_of(d0, 8)
                    for (src, dst, sem) in arrs:
                        copy(src.at[pl.ds(r0, sr), pl.ds(cc * sc, sc)], dst.at[pl.ds(d0, sr), pl.ds(cc * sc, sc)], sem, k % 2)
                        k += 1

        class Stream:
            def __init__(self, arrs, row0, rows, cols, sr, sc, S):
                self.args = (arrs, row0, rows, cols, sr, sc, S)
                self.n = rows // S // sr
                self.pos = 0

            def advance(self, k=None):
                hi = self.n if k is None else min(self.n, self.pos + k)
                _loop(self.pos, hi, lambda j: stream_step(*self.args, j))
                self.pos = hi

        def kv_step(p, slot, s):
            off = pl.multiple_of(p * G, 128)
            cb = s // 2
            half = s - 2 * cb
            c0 = pl.multiple_of(S0 + cb * ksc, 128)
            for b in range(HB):
                r0 = pl.multiple_of(half * (HB * ksr) + b * ksr, 8)
                for t, (src, dst, sem) in enumerate(((kT_hbm, k_v, sem_p.at[0, slot]), (vT_hbm, v_v, sem_p.at[1, slot]))):
                    copy(src.at[pl.ds(off + r0, ksr), pl.ds(c0, ksc)], dst.at[slot, cb, pl.ds(r0, ksr), :], sem, t)

        st_m = Stream([(wmod_hbm, wmod_v, sem_s.at[2])], 0, D, 6 * D, *cfg["m"])
        st_q = Stream([(wq_hbm, wq_v, sem_s.at[3])], 0, D, HD, *cfg["q"])
        o_args = ([(wo_hbm, wo_v, sem_s.at[4])], 0, HD, D) + tuple(cfg["o"])
        assert HD // o_args[6] // o_args[4] == 2 * NS
        gt = cfg.get("gt", 0)
        gua = [(wg_hbm, wgu_v.at[0], sem_gu.at[0]), (wu_hbm, wgu_v.at[1], sem_gu.at[1])]
        st_gu = Stream(gua[::-1] if gt else gua, 0, D, F, *cfg["g"])

        def d_block(j):
            sr, S = cfg["d"]
            for i in range(DR // S // sr):
                stream_step([(wd_hbm, wd_v.at[j], sem_d.at[j])], j * DR, DR, D, sr, D, S, i, drow0=0)

        kv_pos = [0]

        def kv_advance(k=None):
            hi = 2 * NS if k is None else min(2 * NS, kv_pos[0] + k)

            def one(i):
                p = i // NS
                kv_step(p, p, i - p * NS)
            _loop(kv_pos[0], hi, one)
            kv_pos[0] = hi

        cp_c = pltpu.make_async_copy(c_hbm, c_v, sem_s.at[0])
        cp_x = pltpu.make_async_copy(x_hbm, x_v, sem_s.at[1])
        with scope("iss_m"):
            cp_c.start()
            cp_x.start()
            st_m.advance()
            st_q.advance(cfg["q_before_mod"])

        cp_c.wait()
        cf = c_v[...].astype(jnp.float32)
        sc = (cf * jax.nn.sigmoid(cf)).astype(bf16)
        cp_x.wait()
        xf = x_v[...].astype(jnp.float32)
        lnx = _ln(xf)
        with scope("wait_m"):
            wait_buf(wmod_v, sem_s.at[2])
        mods = []
        with scope("mod"):
            for i in range(0, 6, 2):
                if st_q.pos < st_q.n:
                    st_q.advance(2)
                else:
                    kv_advance(4)
                if nocompute:
                    mods.append(wmod_v[0:16, i * D:(i + 2) * D].astype(jnp.float32)[0:1])
                else:
                    mods.append(_dot(sc, wmod_v[:, i * D:(i + 2) * D]))
        sa, ca, ga, sb, cb, gb = [mods[i // 2][:, (i % 2) * D:(i % 2 + 1) * D] for i in range(6)]
        h = (lnx * (1.0 + ca) + sa).astype(bf16)

        with scope("iss_kv0"):
            st_q.advance()
            kv_advance(cfg["kv_before_q"] - kv_pos[0])

        rows = lax.broadcasted_iota(jnp.int32, (8, G), 0)
        cols = lax.broadcasted_iota(jnp.int32, (8, G), 1)
        mask = (cols >= rows * Dh) & (cols < (rows + 1) * Dh)

        with scope("wait_q"):
            wait_buf(wq_v, sem_s.at[3])
        with scope("qall"):
            qper = cfg["q_per_kv"]
            for p0 in range(0, NP, qper):
                kv_advance(2)
                if not nocompute:
                    qp = _dot(h, wq_v[:, p0 * G:(p0 + qper) * G])
                    for p in range(p0, p0 + qper):
                        q_v[p] = jnp.where(mask, jnp.broadcast_to(qp[:, (p - p0) * G:(p - p0 + 1) * G], (8, G)), 0.0)

        with scope("iss_kv01"):
            kv_advance()

        def body(p, carry):
            slot = lax.rem(p, R)
            p2 = jnp.minimum(p + 2, NP - 1)
            slot2 = lax.rem(p2, R)

            def hook(s):
                @pl.when(p + 2 < NP)
                def _():
                    kv_step(p2, slot2, s)

                @pl.when(p + 2 >= NP)
                def _():
                    stream_step(*o_args, (p + 2 - NP) * NS + s)

            with scope("wait_k"):
                wait_buf(k_v.at[slot], sem_p.at[0, slot])
            qb = q_v[p].astype(bf16)

            def s_step(j):
                hook(j)
                if not nocompute:
                    s_v[j] = _dot(qb, k_v[slot, j]) * scale

            with scope("s"):
                _loop(0, NC, s_step)
            with scope("softmax"):
                if not nocompute:
                    sv = [s_v[j] for j in range(NC)]
                    mx = sv[0]
                    for j in range(1, NC):
                        mx = jnp.maximum(mx, sv[j])
                    m = jnp.max(mx, axis=-1, keepdims=True)
                    ev = [jnp.exp(sv[j] - m) for j in range(NC)]
                    tot = ev[0]
                    for j in range(1, NC):
                        tot = tot + ev[j]
                    l = jnp.sum(tot, axis=-1, keepdims=True)
                    for j in range(NC):
                        s_v[j] = ev[j]
            with scope("wait_v"):
                wait_buf(v_v.at[slot], sem_p.at[1, slot])

            def pv_step(j, o):
                hook(NC + j)
                if nocompute:
                    return o
                return o + _dot_nt(s_v[j].astype(bf16), v_v[slot, j])

            with scope("pv"):
                o = lax.fori_loop(0, NC, pv_step, jnp.zeros((8, G), jnp.float32))
            with scope("store_o"):
                if nocompute:
                    q_v[p] = q_v[p] + k_v[slot, 0, 0:16, 0:G].astype(jnp.float32)[0:8]
                else:
                    q_v[p] = jnp.where(mask, o / l, 0.0)
            return carry

        lax.fori_loop(0, NP, body, 0)
        with scope("iss_gu"):
            st_gu.advance()
        with scope("wait_o"):
            wait_buf(wo_v, sem_s.at[4])

        PO = NP // NO
        DO = cfg["d_during_o"]

        def o_step(j, acc):
            if DO:
                @pl.when(j < DO)
                def _():
                    d_block(j)
            if nocompute:
                return acc
            for i in range(PO):
                p = j * PO + i
                off = pl.multiple_of(p * G, 128)
                acc = acc + _dot(q_v[p].astype(bf16), wo_v[pl.ds(off, G), :])
            return acc

        with scope("wo"):
            acc = lax.fori_loop(0, NO, o_step, jnp.zeros((8, D), jnp.float32))
        with scope("iss_d"):
            _loop(DO, ND, d_block)
        with scope("h2"):
            attn = jnp.sum(acc, axis=0, keepdims=True)
            x1 = xf + ga * attn
            h2 = (_ln(x1) * (1.0 + cb) + sb).astype(bf16)

        def gu_step(t):
            wait_buf(wgu_v.at[t], sem_gu.at[t])
            if not nocompute:
                gu_v[t] = _dot(h2, wgu_v[t])

        with scope("gu"):
            _loop(0, 2, gu_step)
        with scope("act"):
            if not nocompute:
                a = _gelu(gu_v[0]) * gu_v[1]
                for j in range(ND):
                    a_v[j] = a[:, j * DR:(j + 1) * DR]

        def d_step(j, y):
            wait_buf(wd_v.at[j], sem_d.at[j])
            if nocompute:
                return y
            return y + _dot(a_v[j].astype(bf16), wd_v[j])

        with scope("d"):
            y = lax.fori_loop(0, ND, d_step, jnp.zeros((1, D), jnp.float32))
        o_ref[...] = (x1 + gb * y).astype(o_ref.dtype)

    return kernel


DEFAULT = dict(kv=(48, 512),
               m=(8, 1920, 8), q=(8, 2048, 8), o=(24, 640, 8),
               q_before_mod=6, kv_before_q=20, q_per_kv=2,
               g=(8, 1536, 5), no=4, nd=6, d=(32, 8), d_during_o=4)


def _build(**over):
    cfg = dict(DEFAULT)
    cfg.update(over)

    def fn(A_x, A_k_cache, A_v_cache, A_wq, A_wo, B_x, B_w_gate, B_w_up, B_w_down, c, w_mod):
        B, Sq, D = A_x.shape
        _, H, Sk, Dh = A_k_cache.shape
        W = min(4096, max(256, Sk // 4))
        F = B_w_gate.shape[1]
        G = 2 * Dh
        R = 3
        ksr, ksc = cfg["kv"]
        NC = W // ksc
        ND = cfg["nd"]
        bf16 = jnp.bfloat16
        kT = jnp.swapaxes(A_k_cache, 2, 3).reshape(H * Dh, Sk)
        vT = jnp.swapaxes(A_v_cache, 2, 3).reshape(H * Dh, Sk)
        x2 = A_x.reshape(1, D)
        kern = make_kernel(D, H, Dh, Sk, W, F, cfg)
        any_spec = pl.BlockSpec(memory_space=pl.ANY)
        out = pl.pallas_call(
            kern,
            out_shape=jax.ShapeDtypeStruct((1, D), A_x.dtype),
            in_specs=[any_spec] * 10,
            out_specs=pl.BlockSpec(memory_space=pltpu.VMEM),
            scratch_shapes=[
                pltpu.VMEM((1, D), bf16),
                pltpu.VMEM((1, D), bf16),
                pltpu.VMEM((D, 6 * D), bf16),
                pltpu.VMEM((D, H * Dh), bf16),
                pltpu.VMEM((R, NC, G, ksc), bf16),
                pltpu.VMEM((R, NC, G, ksc), bf16),
                pltpu.VMEM((H * Dh, D), bf16),
                pltpu.VMEM((2, D, F), bf16),
                pltpu.VMEM((ND, F // ND, D), bf16),
                pltpu.VMEM((H // 2, 8, G), jnp.float32),
                pltpu.VMEM((NC, 8, ksc), jnp.float32),
                pltpu.VMEM((2, 1, F), jnp.float32),
                pltpu.VMEM((ND, 1, F // ND), jnp.float32),
                pltpu.SemaphoreType.DMA((5,)),
                pltpu.SemaphoreType.DMA((2, R)),
                pltpu.SemaphoreType.DMA((2,)),
                pltpu.SemaphoreType.DMA((ND,)),
            ],
            compiler_params=pltpu.CompilerParams(vmem_limit_bytes=100 * 1024 * 1024,
                                                 disable_bounds_checks=True,
                                                 disable_semaphore_checks=True),
        )(x2, c, kT, vT, A_wq, A_wo, B_w_gate, B_w_up, B_w_down, w_mod)
        return out.reshape(B, Sq, D)

    return fn


@jax.jit
def pallas_adaLN_cond__sliding_block_cached__geglu_ffn__decode_kernel(
    A_x: jax.Array,
    A_k_cache: jax.Array,
    A_v_cache: jax.Array,
    A_wq: jax.Array,
    A_wo: jax.Array,
    B_x: jax.Array,
    B_w_gate: jax.Array,
    B_w_up: jax.Array,
    B_w_down: jax.Array,
    c: jax.Array,
    w_mod: jax.Array,
):
    del B_x
    return _build(nd=4, d=(24, 8))(A_x, A_k_cache, A_v_cache, A_wq, A_wo, None, B_w_gate, B_w_up, B_w_down, c, w_mod)
```

```python
import jax
import jax.numpy as jnp
import numpy as np
from jax import lax
from jax.experimental import pallas as pl
from jax.experimental.pallas import tpu as pltpu

_RING = 3
_KV_PIECE = (24, 512)
_MOD_PIECE = (8, 1920, 8)
_WQ_PIECE = (8, 2048, 8)
_WO_PIECE = (24, 640, 8)
_GU_PIECE = (8, 1536, 4)
_WD_PIECE = (24, 8)
_WD_BLOCKS = 4
_WO_STEPS = 4
_Q_STEPS_BEFORE_MOD = 6
_KV_STEPS_BEFORE_Q = 20
_Q_PAIRS_PER_STEP = 2


def _layernorm(x, eps=1e-5):
    m = jnp.mean(x, axis=-1, keepdims=True)
    d = x - m
    v = jnp.mean(d * d, axis=-1, keepdims=True)
    return d / jnp.sqrt(v + eps)


def _gelu_tanh(x):
    c = float(np.sqrt(2.0 / np.pi))
    return 0.5 * x * (1.0 + jnp.tanh(c * (x + 0.044715 * (x * x * x))))


def _dot(a, b):
    return jnp.dot(a, b, preferred_element_type=jnp.float32)


def _dot_nt(a, b):
    return lax.dot_general(a, b, (((1,), (1,)), ((), ())), preferred_element_type=jnp.float32)


def _loop(lo, hi, fn):
    if hi > lo:
        lax.fori_loop(lo, hi, lambda i, carry: (fn(i), carry)[1], 0)


def _make_kernel(D, H, Dh, Sk, W, F):
    bf16 = jnp.bfloat16
    R = _RING
    NP = H // 2
    G = 2 * Dh
    HD = H * Dh
    S0 = Sk - W
    scale = float(Dh) ** -0.5
    ksr, ksc = _KV_PIECE
    NC = W // ksc
    NS = 2 * NC
    HB = G // ksr // 2
    ND = _WD_BLOCKS
    DR = F // ND
    NO = _WO_STEPS
    assert G % 128 == 0 and G % (2 * ksr) == 0 and W % ksc == 0 and NP % NO == 0 and NP >= R
    assert NO <= ND and DR % 128 == 0

    def kernel(x_hbm, c_hbm, kT_hbm, vT_hbm, wq_hbm, wo_hbm, wg_hbm, wu_hbm, wd_hbm, wmod_hbm,
               o_ref,
               x_v, c_v, wmod_v, wq_v, k_v, v_v, wo_v, wgu_v, wd_v, qo_v, s_v, gu_v, a_v,
               sem_w, sem_kv, sem_gu, sem_d):

        def wait_all(buf, sem):
            pltpu.make_async_copy(buf, buf, sem).wait()

        def start(src, dst, sem, priority):
            pltpu.make_async_copy(src, dst, sem).start(priority=priority)

        def stream_step(arrays, row0, rows, cols, sr, sc, regions, j, dst_row0=None):
            reg = rows // regions
            assert reg * regions == rows and reg % sr == 0 and cols % sc == 0 and sr % 8 == 0
            k = 0
            for cc in range(cols // sc):
                for g in range(regions):
                    r = g * reg + j * sr
                    src_r = pl.multiple_of(row0 + r, 8)
                    dst_r = src_r if dst_row0 is None else pl.multiple_of(dst_row0 + r, 8)
                    for (src, dst, sem) in arrays:
                        start(src.at[pl.ds(src_r, sr), pl.ds(cc * sc, sc)],
                              dst.at[pl.ds(dst_r, sr), pl.ds(cc * sc, sc)], sem, k % 2)
                        k += 1

        class Stream:
            def __init__(self, *args):
                self.args = args
                _, _, rows, _, sr, _, regions = args
                self.n = rows // regions // sr
                self.pos = 0

            def advance(self, k=None):
                hi = self.n if k is None else min(self.n, self.pos + k)
                _loop(self.pos, hi, lambda j: stream_step(*self.args, j))
                self.pos = hi

        def kv_step(p, slot, s):
            off = pl.multiple_of(p * G, 128)
            cb = s // 2
            half = s - 2 * cb
            c0 = pl.multiple_of(S0 + cb * ksc, 128)
            for b in range(HB):
                r0 = pl.multiple_of(half * (HB * ksr) + b * ksr, 8)
                for t, (src, dst) in enumerate(((kT_hbm, k_v), (vT_hbm, v_v))):
                    start(src.at[pl.ds(off + r0, ksr), pl.ds(c0, ksc)],
                          dst.at[slot, cb, pl.ds(r0, ksr), :], sem_kv.at[t, slot], t)

        def wd_block(j):
            sr, regions = _WD_PIECE
            for i in range(DR // regions // sr):
                stream_step([(wd_hbm, wd_v.at[j], sem_d.at[j])], j * DR, DR, D, sr, D, regions, i,
                            dst_row0=0)

        mod_stream = Stream([(wmod_hbm, wmod_v, sem_w.at[2])], 0, D, 6 * D, *_MOD_PIECE)
        wq_stream = Stream([(wq_hbm, wq_v, sem_w.at[3])], 0, D, HD, *_WQ_PIECE)
        wo_args = ([(wo_hbm, wo_v, sem_w.at[4])], 0, HD, D) + _WO_PIECE
        assert HD // _WO_PIECE[2] // _WO_PIECE[0] == 2 * NS
        gu_stream = Stream([(wg_hbm, wgu_v.at[0], sem_gu.at[0]), (wu_hbm, wgu_v.at[1], sem_gu.at[1])],
                           0, D, F, *_GU_PIECE)

        kv_pos = [0]

        def kv_advance(k=None):
            hi = 2 * NS if k is None else min(2 * NS, kv_pos[0] + k)

            def one(i):
                p = i // NS
                kv_step(p, p, i - p * NS)

            _loop(kv_pos[0], hi, one)
            kv_pos[0] = hi

        cp_c = pltpu.make_async_copy(c_hbm, c_v, sem_w.at[0])
        cp_x = pltpu.make_async_copy(x_hbm, x_v, sem_w.at[1])
        cp_c.start()
        cp_x.start()
        mod_stream.advance()
        wq_stream.advance(_Q_STEPS_BEFORE_MOD)

        cp_c.wait()
        cf = c_v[...].astype(jnp.float32)
        silu_c = (cf * jax.nn.sigmoid(cf)).astype(bf16)
        cp_x.wait()
        xf = x_v[...].astype(jnp.float32)
        ln_x = _layernorm(xf)
        wait_all(wmod_v, sem_w.at[2])
        mods = []
        for i in range(0, 6, 2):
            if wq_stream.pos < wq_stream.n:
                wq_stream.advance(2)
            else:
                kv_advance(4)
            mods.append(_dot(silu_c, wmod_v[:, i * D:(i + 2) * D]))
        sa, ca, ga, sb, cb_, gb = [mods[i // 2][:, (i % 2) * D:(i % 2 + 1) * D] for i in range(6)]
        h = (ln_x * (1.0 + ca) + sa).astype(bf16)

        wq_stream.advance()
        kv_advance(_KV_STEPS_BEFORE_Q - kv_pos[0])

        rows = lax.broadcasted_iota(jnp.int32, (8, G), 0)
        cols = lax.broadcasted_iota(jnp.int32, (8, G), 1)
        mask = (cols >= rows * Dh) & (cols < (rows + 1) * Dh)

        wait_all(wq_v, sem_w.at[3])
        qn = _Q_PAIRS_PER_STEP
        for p0 in range(0, NP, qn):
            kv_advance(2)
            qp = _dot(h, wq_v[:, p0 * G:(p0 + qn) * G])
            for p in range(p0, p0 + qn):
                qo_v[p] = jnp.where(mask, jnp.broadcast_to(qp[:, (p - p0) * G:(p - p0 + 1) * G], (8, G)), 0.0)
        kv_advance()

        def pair_body(p, carry):
            slot = lax.rem(p, R)
            p2 = jnp.minimum(p + 2, NP - 1)
            slot2 = lax.rem(p2, R)

            def fetch(s):
                @pl.when(p + 2 < NP)
                def _():
                    kv_step(p2, slot2, s)

                @pl.when(p + 2 >= NP)
                def _():
                    stream_step(*wo_args, jnp.clip((p + 2 - NP) * NS + s, 0, 2 * NS - 1))

            wait_all(k_v.at[slot], sem_kv.at[0, slot])
            qb = qo_v[p].astype(bf16)

            def score_step(j):
                fetch(j)
                s_v[j] = _dot(qb, k_v[slot, j]) * scale

            _loop(0, NC, score_step)

            sv = [s_v[j] for j in range(NC)]
            mx = sv[0]
            for j in range(1, NC):
                mx = jnp.maximum(mx, sv[j])
            m = jnp.max(mx, axis=-1, keepdims=True)
            ev = [jnp.exp(sv[j] - m) for j in range(NC)]
            tot = ev[0]
            for j in range(1, NC):
                tot = tot + ev[j]
            l = jnp.sum(tot, axis=-1, keepdims=True)
            for j in range(NC):
                s_v[j] = ev[j]

            wait_all(v_v.at[slot], sem_kv.at[1, slot])

            def pv_step(j, o):
                fetch(NC + j)
                return o + _dot_nt(s_v[j].astype(bf16), v_v[slot, j])

            o = lax.fori_loop(0, NC, pv_step, jnp.zeros((8, G), jnp.float32))
            qo_v[p] = jnp.where(mask, o / l, 0.0)
            return carry

        lax.fori_loop(0, NP, pair_body, 0)

        gu_stream.advance()
        wait_all(wo_v, sem_w.at[4])
        PO = NP // NO

        def wo_step(j, acc):
            wd_block(j)
            for i in range(PO):
                p = j * PO + i
                off = pl.multiple_of(p * G, 128)
                acc = acc + _dot(qo_v[p].astype(bf16), wo_v[pl.ds(off, G), :])
            return acc

        acc = lax.fori_loop(0, NO, wo_step, jnp.zeros((8, D), jnp.float32))
        _loop(NO, ND, wd_block)
        x1 = xf + ga * jnp.sum(acc, axis=0, keepdims=True)
        h2 = (_layernorm(x1) * (1.0 + cb_) + sb).astype(bf16)

        def gu_step(t):
            wait_all(wgu_v.at[t], sem_gu.at[t])
            gu_v[t] = _dot(h2, wgu_v[t])

        _loop(0, 2, gu_step)
        act = _gelu_tanh(gu_v[0]) * gu_v[1]
        for j in range(ND):
            a_v[j] = act[:, j * DR:(j + 1) * DR]

        def wd_step(j, y):
            wait_all(wd_v.at[j], sem_d.at[j])
            return y + _dot(a_v[j].astype(bf16), wd_v[j])

        y = lax.fori_loop(0, ND, wd_step, jnp.zeros((1, D), jnp.float32))
        o_ref[...] = (x1 + gb * y).astype(o_ref.dtype)

    return kernel


@jax.jit
def pallas_adaLN_cond__sliding_block_cached__geglu_ffn__decode_kernel(
    A_x: jax.Array,
    A_k_cache: jax.Array,
    A_v_cache: jax.Array,
    A_wq: jax.Array,
    A_wo: jax.Array,
    B_x: jax.Array,
    B_w_gate: jax.Array,
    B_w_up: jax.Array,
    B_w_down: jax.Array,
    c: jax.Array,
    w_mod: jax.Array,
):
    del B_x
    B, Sq, D = A_x.shape
    _, H, Sk, Dh = A_k_cache.shape
    F = B_w_gate.shape[1]
    W = min(4096, max(256, Sk // 4))
    assert B == 1 and Sq == 1 and A_wq.shape == (D, H * Dh)
    G = 2 * Dh
    ksc = _KV_PIECE[1]
    NC = W // ksc
    bf16 = jnp.bfloat16

    kT = jnp.swapaxes(A_k_cache, 2, 3).reshape(H * Dh, Sk)
    vT = jnp.swapaxes(A_v_cache, 2, 3).reshape(H * Dh, Sk)

    hbm = pl.BlockSpec(memory_space=pl.ANY)
    out = pl.pallas_call(
        _make_kernel(D, H, Dh, Sk, W, F),
        out_shape=jax.ShapeDtypeStruct((1, D), A_x.dtype),
        in_specs=[hbm] * 10,
        out_specs=pl.BlockSpec(memory_space=pltpu.VMEM),
        scratch_shapes=[
            pltpu.VMEM((1, D), bf16),
            pltpu.VMEM((1, D), bf16),
            pltpu.VMEM((D, 6 * D), bf16),
            pltpu.VMEM((D, H * Dh), bf16),
            pltpu.VMEM((_RING, NC, G, ksc), bf16),
            pltpu.VMEM((_RING, NC, G, ksc), bf16),
            pltpu.VMEM((H * Dh, D), bf16),
            pltpu.VMEM((2, D, F), bf16),
            pltpu.VMEM((_WD_BLOCKS, F // _WD_BLOCKS, D), bf16),
            pltpu.VMEM((H // 2, 8, G), jnp.float32),
            pltpu.VMEM((NC, 8, ksc), jnp.float32),
            pltpu.VMEM((2, 1, F), jnp.float32),
            pltpu.VMEM((_WD_BLOCKS, 1, F // _WD_BLOCKS), jnp.float32),
            pltpu.SemaphoreType.DMA((5,)),
            pltpu.SemaphoreType.DMA((2, _RING)),
            pltpu.SemaphoreType.DMA((2,)),
            pltpu.SemaphoreType.DMA((_WD_BLOCKS,)),
        ],
        compiler_params=pltpu.CompilerParams(
            vmem_limit_bytes=64 * 1024 * 1024,
            disable_bounds_checks=True,
            disable_semaphore_checks=True,
        ),
    )(A_x.reshape(1, D), c, kT, vT, A_wq, A_wo, B_w_gate, B_w_up, B_w_down, w_mod)
    return out.reshape(B, Sq, D)
```
